```python
import jax
import jax.numpy as jnp

def _softmax(x, axis=-1):
    return jax.nn.softmax(x, axis=axis)
def _gelu(x):
    return jax.nn.gelu(x, approximate=True)
def _silu(x):
    return jax.nn.silu(x)
def _sigmoid(x):
    return jax.nn.sigmoid(x)
def _layernorm(x, axis=-1, eps=1e-5):
    m = jnp.mean(x, axis=axis, keepdims=True)
    v = jnp.var(x, axis=axis, keepdims=True)
    return (x - m) / jnp.sqrt(v + eps)
def _scatter_add(tgt, idx, src, axis=0):
    return tgt.at[idx].add(src)
def _segment_sum(src, seg, n):
    return jax.ops.segment_sum(src, seg, n)
class _Rng:
    def __init__(self, key):
        self._k = key
    def _next(self):
        self._k, sub = jax.random.split(self._k)
        return sub
    def normal(self, shape):
        return jax.random.normal(self._next(), shape, dtype=jnp.bfloat16)
    def randint(self, lo, hi, shape):
        return jax.random.randint(self._next(), shape, lo, hi, dtype=jnp.int32)
    def uniform(self, shape, lo=0.0, hi=1.0):
        return jax.random.uniform(self._next(), shape, jnp.bfloat16, lo, hi)
    def permutation(self, n):
        return jax.random.permutation(self._next(), n)


kernel_name = 'recurrent_scan__sliding_block_cached__mixer_s_mlp__decode'

def setup_inputs():
    _rng = _Rng(jax.random.key(int.from_bytes(__import__("os").urandom(4), "little")))
    _w = (lambda a: (lambda t: t.astype(jnp.bfloat16) if jnp.issubdtype(t.dtype, jnp.floating) else t)(jnp.asarray(a)))
    def _A_setup():
        B, Sq, D = 1, 1, 512
        Hq, Hkv, Sk, Dh = 32, 32, 32768, 128
        assert Hq % Hkv == 0, (Hq, Hkv)
        return {
            "x": _w((lambda *s: _rng.normal(s) * 0.05)(B, Sq, D)),
            "k_cache": _w((lambda *s: _rng.normal(s) * 0.05)(B, Hkv, Sk, Dh)),
            "v_cache": _w((lambda *s: _rng.normal(s) * 0.05)(B, Hkv, Sk, Dh)),
            "wq": _w((lambda *s: _rng.normal(s) * 0.05)(D, Hq * Dh) * (D ** -0.5)),
            "wo": _w((lambda *s: _rng.normal(s) * 0.05)(Hq * Dh, D) * ((Hq * Dh) ** -0.5)),
        }
    _A_in = _A_setup()

    def _B_setup():
        B, S, D, F = 1, 1, 512, 1376
        return {
            "x":  _w((lambda *s: _rng.normal(s) * 0.05)(B, S, D)),
            "w1": _w((lambda *s: _rng.normal(s) * 0.05)(D, D) * (D ** -0.5)),
            "w2": _w((lambda *s: _rng.normal(s) * 0.05)(D, D) * (D ** -0.5)),
            "w3": _w((lambda *s: _rng.normal(s) * 0.05)(D, F) * (D ** -0.5)),
            "w4": _w((lambda *s: _rng.normal(s) * 0.05)(F, D) * (F ** -0.5)),
        }
    _B_in = _B_setup()

    return {
        "A_x": _A_in["x"],
        "A_k_cache": _A_in["k_cache"],
        "A_v_cache": _A_in["v_cache"],
        "A_wq": _A_in["wq"],
        "A_wo": _A_in["wo"],
        "B_x": _B_in["x"],
        "B_w1": _B_in["w1"],
        "B_w2": _B_in["w2"],
        "B_w3": _B_in["w3"],
        "B_w4": _B_in["w4"],
    }

def reference(A_x, A_k_cache, A_v_cache, A_wq, A_wo, B_x, B_w1, B_w2, B_w3, B_w4):
    def _A_ref(x, k_cache, v_cache, wq, wo):
        B, Sq, D = x.shape
        Hq, Dh = 32, 128
        Hkv, Sk = k_cache.shape[1], k_cache.shape[2]
        W = min(4096, max(256, Sk // 4))
        rep = Hq // Hkv
        q = (lambda x, *d: x.transpose(*d))((x @ wq).reshape(B, Sq, Hq, Dh), 0, 2, 1, 3)
        k = jnp.repeat(k_cache[:, :, Sk - W:, :], rep, axis=1)
        v = jnp.repeat(v_cache[:, :, Sk - W:, :], rep, axis=1)
        scores = jnp.einsum("bhqd,bhkd->bhqk", q, k) * (Dh ** -0.5)
        p = _softmax(scores, axis=-1)
        o = jnp.einsum("bhqk,bhkd->bhqd", p, v)
        return (lambda x, *d: x.transpose(*d))(o, 0, 2, 1, 3).reshape(B, Sq, Hq * Dh) @ wo

    def _B_ref(x, w1, w2, w3, w4):
        B, S, D = x.shape
        h = _gelu(_layernorm(x, axis=-1) @ w1)
        c = D // 4
        g0 = jnp.pad(h[:, :, 0*c:1*c], ((0, 0), (1, 0), (0, 0)))[:, :S, :]
        g1 = jnp.pad(h[:, :, 1*c:2*c], ((0, 0), (0, 1), (0, 0)))[:, 1:, :]
        g2 = jnp.pad(h[:, :, 2*c:3*c], ((0, 0), (2, 0), (0, 0)))[:, :S, :]
        g3 = jnp.pad(h[:, :, 3*c:   ], ((0, 0), (0, 2), (0, 0)))[:, 2:, :]
        hs = jnp.concatenate([g0, g1, g2, g3], axis=-1) @ w2
        x1 = x + hs
        h2 = _gelu(_layernorm(x1, axis=-1) @ w3) @ w4
        return x1 + h2

    x = A_x
    xn = _layernorm(x, axis=-1)
    s = _A_ref(xn, A_k_cache, A_v_cache, A_wq, A_wo)
    g = _silu(_B_ref(xn, B_w1, B_w2, B_w3, B_w4))
    return x + s * g
```

```python
import jax
import jax.numpy as jnp
from jax import lax
import jax.experimental.pallas as pl
import jax.experimental.pallas.tpu as pltpu

BF, F32 = jnp.bfloat16, jnp.float32
DH = 128
NT = (((1,), (1,)), ((), ()))
NN = (((1,), (0,)), ((), ()))

ROWS = 64
LOOK = 2
WR = 32
WQC = 1024
UNROLL = 4
FSPLIT = 1024


def _layernorm(x):
    m = jnp.mean(x, axis=-1, keepdims=True)
    d = x - m
    v = jnp.mean(d * d, axis=-1, keepdims=True)
    return d / jnp.sqrt(v + 1e-5)


def _dot(a, b, dims):
    return lax.dot_general(a, b, dims, preferred_element_type=F32)


def _kernel(x_hbm, k_hbm, v_hbm, wq_hbm, wo_hbm, w3t_hbm, w4_hbm, o_ref,
            xb, kb, vb, wqb, wob, w3b, w4b, qb, ksem, vsem, msem):
    H, W, _ = kb.shape
    SK = k_hbm.shape[2]
    F, D = w4b.shape
    ns = LOOK + 1
    mo = pl.multiple_of
    copy = pltpu.make_async_copy

    def start_head(h, slot):
        def it(jj, c):
            for u in range(UNROLL):
                r0 = mo((jj * UNROLL + u) * ROWS, ROWS)
                copy(k_hbm.at[0, h, pl.ds(SK - W + r0, ROWS)], kb.at[h, pl.ds(r0, ROWS)],
                     ksem.at[slot]).start(priority=0)
                copy(v_hbm.at[0, h, pl.ds(SK - W + r0, ROWS)], vb.at[h, pl.ds(r0, ROWS)],
                     vsem.at[slot]).start(priority=1)
            return c
        lax.fori_loop(0, W // (ROWS * UNROLL), it, 0)
        for j in range(DH // WR):
            copy(wo_hbm.at[pl.ds(mo(h * DH + j * WR, WR), WR)], wob.at[h, pl.ds(j * WR, WR)],
                 vsem.at[slot]).start(priority=j % 2)

    def start_rows(src, dst, lo, hi, sem):
        n = (hi - lo) // WR

        def it(jj, c):
            for u in range(2):
                r0 = mo(lo + (2 * jj + u) * WR, WR)
                copy(src.at[pl.ds(r0, WR)], dst.at[pl.ds(r0, WR)], sem).start(priority=u)
            return c
        lax.fori_loop(0, n // 2, it, 0)
        if n % 2:
            copy(src.at[pl.ds(hi - WR, WR)], dst.at[pl.ds(hi - WR, WR)], sem).start(priority=0)

    def wait_rows(src, dst, lo, hi, sem):
        copy(src.at[pl.ds(lo, hi - lo)], dst.at[pl.ds(lo, hi - lo)], sem).wait()

    cx = copy(x_hbm.at[0], xb, msem.at[0])
    cx.start()

    def wq_it(jj, c):
        r0 = mo(jj * 16, 16)
        for u in range(H * DH // WQC):
            copy(wq_hbm.at[pl.ds(r0, 16), pl.ds(u * WQC, WQC)],
                 wqb.at[pl.ds(r0, 16), pl.ds(u * WQC, WQC)], msem.at[1]).start(priority=u % 2)
        return c
    lax.fori_loop(0, D // 16, wq_it, 0)

    def h_it(h, c):
        start_head(h, h)
        return c
    lax.fori_loop(0, LOOK, h_it, 0)

    cx.wait()
    x = jnp.broadcast_to(xb[...].astype(F32), (8, D))
    xn = _layernorm(x).astype(BF)
    x1 = xn.astype(F32)
    xn2 = _layernorm(x1).astype(BF)
    copy(wq_hbm, wqb, msem.at[1]).wait()
    q = _dot(xn, wqb[...], NN)
    for h in range(H):
        qb[h] = q[:, h * DH:(h + 1) * DH]

    def body(h, acc):
        slot = lax.rem(h, ns)

        @pl.when(h + LOOK < H)
        def _():
            start_head(h + LOOK, lax.rem(h + LOOK, ns))

        @pl.when(h + LOOK == H)
        def _():
            start_rows(w3t_hbm, w3b, 0, F, msem.at[2])

        @pl.when(h + LOOK == H + 1)
        def _():
            start_rows(w4_hbm, w4b, 0, FSPLIT, msem.at[3])
            start_rows(w4_hbm, w4b, FSPLIT, F, msem.at[4])

        window = pl.ds(SK - W, W)
        copy(k_hbm.at[0, h, window], kb.at[h], ksem.at[slot]).wait()
        s = _dot(qb[h].astype(BF), kb[h], NT) * (DH ** -0.5)
        m = jnp.max(s, axis=-1, keepdims=True)
        p = jnp.exp(s - m)
        l = jnp.sum(p, axis=-1, keepdims=True)
        copy(v_hbm.at[0, h, window], vb.at[h], vsem.at[slot]).wait()
        copy(wo_hbm.at[pl.ds(mo(h * DH, DH), DH)], wob.at[h], vsem.at[slot]).wait()
        o = _dot(p.astype(BF), vb[h], NN) / l
        return acc + _dot(o.astype(BF), wob[h], NN)

    s = lax.fori_loop(0, H, body, jnp.zeros((8, D), F32))

    wait_rows(w3t_hbm, w3b, 0, F, msem.at[2])
    u = jax.nn.gelu(_dot(xn2, w3b[...], NT), approximate=True).astype(BF)
    wait_rows(w4_hbm, w4b, 0, FSPLIT, msem.at[3])
    y = x1 + _dot(u[:, :FSPLIT], w4b[pl.ds(0, FSPLIT), :], NN)
    wait_rows(w4_hbm, w4b, FSPLIT, F, msem.at[4])
    y = y + _dot(u[:, FSPLIT:], w4b[pl.ds(FSPLIT, F - FSPLIT), :], NN)
    g = y * jax.nn.sigmoid(y)
    o_ref[0] = (x + s * g)[0:1].astype(o_ref.dtype)


@jax.jit
def pallas_recurrent_scan__sliding_block_cached__mixer_s_mlp__decode_kernel(
    A_x: jax.Array,
    A_k_cache: jax.Array,
    A_v_cache: jax.Array,
    A_wq: jax.Array,
    A_wo: jax.Array,
    B_x: jax.Array,
    B_w1: jax.Array,
    B_w2: jax.Array,
    B_w3: jax.Array,
    B_w4: jax.Array,
):
    B, Sq, D = A_x.shape
    _, H, SK, _ = A_k_cache.shape
    F = B_w4.shape[0]
    W = min(4096, max(256, SK // 4))
    assert (B, Sq) == (1, 1) and A_wq.shape == (D, H * DH)
    assert W % (ROWS * UNROLL) == 0 and F % WR == 0 and F > FSPLIT

    return pl.pallas_call(
        _kernel,
        in_specs=[pl.BlockSpec(memory_space=pl.ANY)] * 7,
        out_specs=pl.BlockSpec(memory_space=pltpu.VMEM),
        out_shape=jax.ShapeDtypeStruct((1, 1, D), A_x.dtype),
        scratch_shapes=[
            pltpu.VMEM((1, D), BF),
            pltpu.VMEM((H, W, DH), BF),
            pltpu.VMEM((H, W, DH), BF),
            pltpu.VMEM((D, H * DH), BF),
            pltpu.VMEM((H, DH, D), BF),
            pltpu.VMEM((F, D), BF),
            pltpu.VMEM((F, D), BF),
            pltpu.VMEM((H, 8, DH), F32),
            pltpu.SemaphoreType.DMA((LOOK + 1,)),
            pltpu.SemaphoreType.DMA((LOOK + 1,)),
            pltpu.SemaphoreType.DMA((5,)),
        ],
        compiler_params=pltpu.CompilerParams(vmem_limit_bytes=100 * 2**20),
    )(A_x, A_k_cache, A_v_cache, A_wq, A_wo, B_w3.T, B_w4)
```
